```python
import os as _os
_os.environ.setdefault("JAX_PLATFORMS", "cpu")
import jax
import jax.numpy as jnp

def _softmax(x, axis=-1):
    return jax.nn.softmax(x, axis=axis)
def _gelu(x):
    return jax.nn.gelu(x, approximate=True)
def _silu(x):
    return jax.nn.silu(x)
def _sigmoid(x):
    return jax.nn.sigmoid(x)
def _layernorm(x, axis=-1, eps=1e-5):
    m = jnp.mean(x, axis=axis, keepdims=True)
    v = jnp.var(x, axis=axis, keepdims=True)
    return (x - m) / jnp.sqrt(v + eps)
def _scatter_add(tgt, idx, src, axis=0):
    return tgt.at[idx].add(src)
def _segment_sum(src, seg, n):
    return jax.ops.segment_sum(src, seg, n)
class _Rng:
    def __init__(self, key):
        self._k = key
    def _next(self):
        self._k, sub = jax.random.split(self._k)
        return sub
    def normal(self, shape):
        return jax.random.normal(self._next(), shape, dtype=jnp.bfloat16)
    def randint(self, lo, hi, shape):
        return jax.random.randint(self._next(), shape, lo, hi, dtype=jnp.int32)
    def uniform(self, shape, lo=0.0, hi=1.0):
        return jax.random.uniform(self._next(), shape, jnp.bfloat16, lo, hi)
    def permutation(self, n):
        return jax.random.permutation(self._next(), n)


kernel_name = 'gated_mix__linear_attn_block__mixer_s_mlp__prompt'

def setup_inputs():
    _rng = _Rng(jax.random.key(int.from_bytes(__import__("os").urandom(4), "little")))
    _w = (lambda a: (lambda t: t.astype(jnp.bfloat16) if jnp.issubdtype(t.dtype, jnp.floating) else t)(jnp.asarray(a)))
    def _A_setup():
        B, S, D = 1, 2048, 640
        return {
            "x": _w((lambda *s: _rng.normal(s) * 0.05)(B, S, D)),
            "wqkv": _w((lambda *s: _rng.normal(s) * 0.8)(D, 3 * D)),
            "wo": _w((lambda *s: _rng.normal(s) * 0.1)(D, D)),
        }
    _A_in = _A_setup()

    def _B_setup():
        B, S, D, F = 1, 2048, 640, 1728
        return {
            "x":  _w((lambda *s: _rng.normal(s) * 0.05)(B, S, D)),
            "w1": _w((lambda *s: _rng.normal(s) * 0.2)(D, D) * (D ** -0.5)),
            "w2": _w((lambda *s: _rng.normal(s) * 0.2)(D, D) * (D ** -0.5)),
            "w3": _w((lambda *s: _rng.normal(s) * 0.2)(D, F) * (D ** -0.5)),
            "w4": _w((lambda *s: _rng.normal(s) * 0.2)(F, D) * (F ** -0.5)),
        }
    _B_in = _B_setup()

    return {
        "A_x": _A_in["x"],
        "A_wqkv": _A_in["wqkv"],
        "A_wo": _A_in["wo"],
        "B_x": _B_in["x"],
        "B_w1": _B_in["w1"],
        "B_w2": _B_in["w2"],
        "B_w3": _B_in["w3"],
        "B_w4": _B_in["w4"],
        "gate_w": _w((lambda *s: _rng.normal(s) * 0.05)(640) * 16.0),
    }

def reference(A_x, A_wqkv, A_wo, B_x, B_w1, B_w2, B_w3, B_w4, gate_w):
    def _A_ref(x, wqkv, wo):
        B, S, D = x.shape
        H = 32; Dh = D // H
        qkv = (lambda x, *d: x.transpose(*d))((x @ wqkv).reshape(B, S, 3, H, Dh), 2, 0, 3, 1, 4)
        q, k, v = qkv[0], qkv[1], qkv[2]
        phi = lambda t: jnp.where(t > 0, t + 1, jnp.exp(t)) + 1e-6
        pq, pk = phi(q), phi(k)
        kv = jnp.einsum("bhsd,bhse->bhde", pk, v)
        z = jnp.einsum("bhsd->bhd", pk)
        num = jnp.einsum("bhqd,bhde->bhqe", pq, kv)
        den = jnp.einsum("bhqd,bhd->bhq", pq, z)[..., None] + 1e-6
        o = num / den
        return (lambda x, *d: x.transpose(*d))(o, 0, 2, 1, 3).reshape(B, S, D) @ wo

    def _B_ref(x, w1, w2, w3, w4):
        B, S, D = x.shape
        h = _gelu(_layernorm(x, axis=-1) @ w1)
        c = D // 4
        g0 = jnp.pad(h[:, :, 0*c:1*c], ((0, 0), (1, 0), (0, 0)))[:, :S, :]
        g1 = jnp.pad(h[:, :, 1*c:2*c], ((0, 0), (0, 1), (0, 0)))[:, 1:, :]
        g2 = jnp.pad(h[:, :, 2*c:3*c], ((0, 0), (2, 0), (0, 0)))[:, :S, :]
        g3 = jnp.pad(h[:, :, 3*c:   ], ((0, 0), (0, 2), (0, 0)))[:, 2:, :]
        hs = jnp.concatenate([g0, g1, g2, g3], axis=-1) @ w2
        x1 = x + hs
        h2 = _gelu(_layernorm(x1, axis=-1) @ w3) @ w4
        return x1 + h2

    x = A_x
    g = _sigmoid((x * gate_w).sum(-1, keepdims=True))
    a = _A_ref(x, A_wqkv, A_wo)
    b = _B_ref(x, B_w1, B_w2, B_w3, B_w4)
    return g * a + (1 - g) * b
```

```python
import functools
import jax
import jax.numpy as jnp
from jax import lax
from jax.experimental import pallas as pl
from jax.experimental.pallas import tpu as pltpu

S = 2048
D = 640
F = 1728
H = 32
DH = 20
TM = 256
NT = S // TM
PAD = 8
BF = jnp.bfloat16
F32 = jnp.float32


def _dot(a, b):
    return jnp.dot(a, b, preferred_element_type=F32)


def _dot_nt(a, b):
    return lax.dot_general(a, b, (((1,), (1,)), ((), ())), preferred_element_type=F32)


def _gelu(x):
    c = 0.7978845608028654
    return 0.5 * x * (1.0 + jnp.tanh(c * (x + 0.044715 * (x * x * x))))


def _phi(t):
    return jnp.where(t > 0, t + 1.0, jnp.exp(t)) + 1e-6


def _ln(x):
    m = jnp.mean(x, axis=-1, keepdims=True)
    xc = x - m
    v = jnp.mean(xc * xc, axis=-1, keepdims=True)
    return xc * lax.rsqrt(v + 1e-5)


def _head(idx):
    return (idx * 3277) >> 16


def _kernel(ax_hbm, wqkv_hbm, wo_hbm, w1_hbm, w2_hbm, w3t_hbm, w4_hbm, gw_ref,
            out_hbm,
            xa, wqkv, wo, w1, w2, w3t, w4, wkT, hbuf, pacc, zacc, mmat, zs, emat, obuf,
            sem_xa, sem_w, sem_o):
    def xa_cp(i):
        return pltpu.make_async_copy(ax_hbm.at[0, pl.ds(i * TM, TM), :], xa.at[pl.ds(i * TM, TM), :], sem_xa.at[i])

    w_cps = [
        pltpu.make_async_copy(w1_hbm, w1, sem_w.at[0]),
        pltpu.make_async_copy(wqkv_hbm.at[:, pl.ds(D, D)], wqkv.at[:, pl.ds(D, D)], sem_w.at[1]),
        pltpu.make_async_copy(wqkv_hbm.at[:, pl.ds(2 * D, D)], wqkv.at[:, pl.ds(2 * D, D)], sem_w.at[2]),
        pltpu.make_async_copy(wo_hbm, wo, sem_w.at[3]),
        pltpu.make_async_copy(wqkv_hbm.at[:, pl.ds(0, D)], wqkv.at[:, pl.ds(0, D)], sem_w.at[4]),
        pltpu.make_async_copy(w2_hbm, w2, sem_w.at[5]),
        pltpu.make_async_copy(w3t_hbm, w3t, sem_w.at[6]),
        pltpu.make_async_copy(w4_hbm, w4, sem_w.at[7]),
    ]
    xa_cp(0).start()
    w_cps[0].start()
    w_cps[1].start()
    for i in range(1, NT):
        xa_cp(i).start()
    for c in w_cps[2:]:
        c.start()

    hbuf[0:PAD, :] = jnp.zeros((PAD, D), F32)
    hbuf[PAD + S:PAD + S + PAD, :] = jnp.zeros((PAD, D), F32)
    pacc[...] = jnp.zeros(pacc.shape, F32)
    zacc[...] = jnp.zeros(zacc.shape, F32)
    ej = lax.broadcasted_iota(jnp.int32, (128, D), 0)
    ee = lax.broadcasted_iota(jnp.int32, (128, D), 1)
    emat[...] = jnp.where((ej < 64) & ((ej & 31) == _head(ee)), 1.0, 0.0).astype(BF)

    w_cps[0].wait()
    w_cps[1].wait()
    wkT[...] = wqkv[:, D:2 * D].T

    def phase1(i, carry):
        r0 = pl.multiple_of(i * TM, TM)
        xa_cp(i).wait()
        xat = xa[pl.ds(r0, TM), :]
        h = _gelu(_dot(_ln(xat.astype(F32)).astype(BF), w1[...]))
        hbuf[pl.ds(PAD + r0, TM), :] = h
        pkT = _phi(_dot_nt(wkT[...], xat))
        zp = pkT[:, 0:128]
        for c in range(1, TM // 128):
            zp = zp + pkT[:, c * 128:(c + 1) * 128]
        zacc[...] += zp
        pacc[...] += _dot(pkT.astype(BF), xat)
        return carry

    lax.fori_loop(0, NT, phase1, 0)

    for c in w_cps[2:]:
        c.wait()

    kv = _dot(pacc[...].astype(BF), wqkv[:, 2 * D:3 * D])
    rd = lax.broadcasted_iota(jnp.int32, (D, D), 0)
    ce = lax.broadcasted_iota(jnp.int32, (D, D), 1)
    kv = jnp.where(_head(rd) == _head(ce), kv, 0.0).astype(BF)
    mmat[...] = _dot(kv, wo[...]).astype(BF)
    z = jnp.sum(zacc[...], axis=1, keepdims=True)
    zd = lax.broadcasted_iota(jnp.int32, (D, 128), 0)
    zj = lax.broadcasted_iota(jnp.int32, (D, 128), 1)
    zs[...] = jnp.where((zj < 64) & ((zj & 31) == _head(zd)), z, 0.0).astype(BF)

    def out_cp(i, slot):
        return pltpu.make_async_copy(obuf.at[slot], out_hbm.at[0, pl.ds(i * TM, TM), :], sem_o.at[slot])

    gw = gw_ref[...].astype(F32).reshape(1, D)

    def phase2(i, carry):
        r0 = pl.multiple_of(i * TM, TM)
        slot = i % 2
        xat = xa[pl.ds(r0, TM), :]
        xf = xat.astype(F32)
        pq = _phi(_dot(xat, wqkv[:, 0:D]))
        den = _dot(pq.astype(BF), zs[...]) + 1e-6
        g = jax.nn.sigmoid(jnp.sum(xf * gw, axis=-1, keepdims=True))
        rec = g / den
        hi = rec.astype(BF).astype(F32)
        lane = lax.broadcasted_iota(jnp.int32, (TM, 128), 1)
        hl = jnp.where(lane < 32, hi, jnp.where(lane < 64, rec - hi, 0.0)).astype(BF)
        r = (pq * _dot(hl, emat[...])).astype(BF)
        a = _dot(r, mmat[...])

        hw = hbuf[pl.ds(r0, TM + 2 * PAD), :]
        col = lax.broadcasted_iota(jnp.int32, (TM, D), 1)
        g0 = hw[PAD - 1:PAD - 1 + TM, :]
        g1 = hw[PAD + 1:PAD + 1 + TM, :]
        g2 = hw[PAD - 2:PAD - 2 + TM, :]
        g3 = hw[PAD + 2:PAD + 2 + TM, :]
        hs_in = jnp.where(col < 160, g0, jnp.where(col < 320, g1, jnp.where(col < 480, g2, g3))).astype(BF)
        x1 = xf + _dot(hs_in, w2[...])
        h2 = _gelu(_dot_nt(_ln(x1).astype(BF), w3t[...])).astype(BF)
        y = _dot(h2, w4[...])
        o = a + (1.0 - g) * (x1 + y)

        @pl.when(i >= 2)
        def _():
            out_cp(i - 2, slot).wait()

        obuf[slot] = o.astype(BF)
        out_cp(i, slot).start()
        return carry

    lax.fori_loop(0, NT, phase2, 0)
    out_cp(NT - 2, (NT - 2) % 2).wait()
    out_cp(NT - 1, (NT - 1) % 2).wait()


@jax.jit
def pallas_gated_mix__linear_attn_block__mixer_s_mlp__prompt_kernel(A_x, A_wqkv, A_wo, B_x, B_w1, B_w2, B_w3, B_w4, gate_w):
    hbm = pl.BlockSpec(memory_space=pltpu.HBM)
    return pl.pallas_call(
        _kernel,
        out_shape=jax.ShapeDtypeStruct((1, S, D), BF),
        in_specs=[hbm] * 7 + [pl.BlockSpec(memory_space=pltpu.VMEM)],
        out_specs=hbm,
        scratch_shapes=[
            pltpu.VMEM((S, D), BF),
            pltpu.VMEM((D, 3 * D), BF), pltpu.VMEM((D, D), BF), pltpu.VMEM((D, D), BF), pltpu.VMEM((D, D), BF),
            pltpu.VMEM((F, D), BF), pltpu.VMEM((F, D), BF),
            pltpu.VMEM((D, D), BF),
            pltpu.VMEM((S + 2 * PAD, D), F32),
            pltpu.VMEM((D, D), F32), pltpu.VMEM((D, 128), F32),
            pltpu.VMEM((D, D), BF), pltpu.VMEM((D, 128), BF), pltpu.VMEM((128, D), BF),
            pltpu.VMEM((2, TM, D), BF),
            pltpu.SemaphoreType.DMA((NT,)),
            pltpu.SemaphoreType.DMA((8,)), pltpu.SemaphoreType.DMA((2,)),
        ],
        compiler_params=pltpu.CompilerParams(vmem_limit_bytes=100 * 1024 * 1024),
        name="gmix",
    )(A_x, A_wqkv, A_wo, B_w1, B_w2, B_w3.T, B_w4, gate_w)
```

```python
import functools
import jax
import jax.numpy as jnp
from jax import lax
from jax.experimental import pallas as pl
from jax.experimental.pallas import tpu as pltpu

S = 2048
D = 640
F = 1728
TM = 256
NT = S // TM
PAD = 8
NSPLIT = 384
U = 2
MODE = 'plain'
BF = jnp.bfloat16
F32 = jnp.float32
EPS = 1e-5

BAND = ((0, 144), (112, 272), (240, 400), (368, 528), (496, 640))


def _dot(a, b):
    return jnp.dot(a, b, preferred_element_type=F32)


def _dot_nt(a, b):
    return lax.dot_general(a, b, (((1,), (1,)), ((), ())), preferred_element_type=F32)


def _gelu(x):
    c = 0.7978845608028654
    return 0.5 * x * (1.0 + jnp.tanh(c * (x + 0.044715 * (x * x * x))))


def _phi(t):
    return jnp.where(t > 0, t + 1.0, jnp.exp(t)) + 1e-6


def _stats(x):
    m = jnp.mean(x, axis=-1, keepdims=True)
    xc = x - m
    v = jnp.mean(xc * xc, axis=-1, keepdims=True)
    return m, lax.rsqrt(v + EPS)


def _head(idx):
    return (idx * 3277) >> 16


def _kernel(ax_hbm, wqkv_hbm, wo_hbm, w1_hbm, w2_hbm, w3t_hbm, w4_hbm, gw_hbm,
            out_hbm,
            xa, wqkv, wo, w1, w2, w3t, w4, gw_ref, wkT, hbuf, pacc, zacc, mmat, zs, obuf,
            sem_xa, sem_w, sem_o):
    def x_cp(n, lo, hi):
        return pltpu.make_async_copy(ax_hbm.at[0, pl.ds(lo, hi - lo), :], xa.at[pl.ds(lo, hi - lo), :], sem_xa.at[n])

    x01_cp = x_cp(0, 0, 2 * TM)
    x23_cp = x_cp(1, 2 * TM, 4 * TM)
    x47_cp = x_cp(2, 4 * TM, 8 * TM)
    w1_cp = pltpu.make_async_copy(w1_hbm, w1, sem_w.at[7])
    gw_cp = pltpu.make_async_copy(gw_hbm, gw_ref, sem_w.at[8])
    wk_cp = pltpu.make_async_copy(wqkv_hbm.at[:, pl.ds(D, D)], wqkv.at[:, pl.ds(D, D)], sem_w.at[0])
    wv_cp = pltpu.make_async_copy(wqkv_hbm.at[:, pl.ds(2 * D, D)], wqkv.at[:, pl.ds(2 * D, D)], sem_w.at[1])
    wo_cp = pltpu.make_async_copy(wo_hbm, wo, sem_w.at[2])
    w_cps = [
        pltpu.make_async_copy(wqkv_hbm.at[:, pl.ds(0, D)], wqkv.at[:, pl.ds(0, D)], sem_w.at[3]),
        pltpu.make_async_copy(w2_hbm, w2, sem_w.at[4]),
        pltpu.make_async_copy(w3t_hbm, w3t, sem_w.at[5]),
        pltpu.make_async_copy(w4_hbm, w4, sem_w.at[6]),
    ]
    wk_cp.start()
    x01_cp.start()
    gw_cp.start()

    hbuf[0:PAD, :] = jnp.zeros((PAD, D), F32)
    hbuf[PAD + S:PAD + S + PAD, :] = jnp.zeros((PAD, D), F32)

    def xt(i):
        return xa[i * TM:(i + 1) * TM, :]

    def stage_ln(i):
        x = xt(i).astype(F32)
        m, rs = _stats(x)
        return (x * rs - m * rs).astype(BF)

    def stage_b(i, ln):
        hbuf[PAD + i * TM:PAD + (i + 1) * TM, :] = _gelu(_dot(ln, w1[...]))

    T2 = 2 * TM

    def stage_k(i):
        pkT = _phi(_dot_nt(wkT[...], xa[i * T2:(i + 1) * T2, :]))
        zp = pkT[:, 0:128]
        for c in range(1, T2 // 128):
            zp = zp + pkT[:, c * 128:(c + 1) * 128]
        if i == 0:
            zacc[...] = zp
        else:
            zacc[...] += zp
        return pkT.astype(BF)

    def stage_p(i, pk):
        t = _dot(pk, xa[i * T2:(i + 1) * T2, :])
        if i == 0:
            pacc[...] = t
        else:
            pacc[...] += t

    def stage_lb(i):
        stage_b(i, stage_ln(i))

    wk_cp.wait()
    x23_cp.start()
    x47_cp.start()
    wkT[...] = wqkv[:, D:2 * D].T
    x01_cp.wait()
    w1_cp.start()
    wv_cp.start()
    wo_cp.start()
    pk0 = stage_k(0)
    x23_cp.wait()
    for c in w_cps:
        c.start()
    stage_p(0, pk0)
    pk1 = stage_k(1)
    x47_cp.wait()
    w1_cp.wait()
    wv_cp.wait()
    wo_cp.wait()
    stage_p(1, pk1)
    pk2 = stage_k(2)
    stage_lb(0)
    stage_lb(1)
    stage_p(2, pk2)
    pk3 = stage_k(3)
    stage_lb(2)
    stage_lb(3)
    stage_p(3, pk3)
    stage_lb(4)
    stage_lb(5)

    kvs = []
    for j, (lo, hi) in enumerate(BAND):
        kv = _dot(pacc[lo:hi, :].astype(BF), wqkv[:, 2 * D + 128 * j:2 * D + 128 * (j + 1)])
        rd = lax.broadcasted_iota(jnp.int32, (hi - lo, 128), 0) + lo
        ce = lax.broadcasted_iota(jnp.int32, (hi - lo, 128), 1) + 128 * j
        kvs.append(jnp.where(_head(rd) == _head(ce), kv, 0.0).astype(BF))
    stage_lb(6)
    ms = [_dot(kvs[j], wo[128 * j:128 * (j + 1), :]) for j in range(5)]
    for j, (lo, hi) in enumerate(BAND):
        a = lo if j == 0 else BAND[j - 1][1]
        b = hi if j == len(BAND) - 1 else BAND[j + 1][0]
        mmat[a:b, :] = ms[j][a - lo:b - lo, :].astype(BF)
        if j + 1 < len(BAND):
            lo2 = BAND[j + 1][0]
            mmat[b:hi, :] = (ms[j][b - lo:hi - lo, :] + ms[j + 1][b - lo2:hi - lo2, :]).astype(BF)
    stage_lb(7)
    z = jnp.sum(zacc[...], axis=1, keepdims=True)
    zd = lax.broadcasted_iota(jnp.int32, (D, 128), 0)
    zj = lax.broadcasted_iota(jnp.int32, (D, 128), 1)
    zs[...] = jnp.where(zj == _head(zd), z, 0.0).astype(BF)

    for c in w_cps:
        c.wait()
    gw_cp.wait()

    def out_cp(i):
        return pltpu.make_async_copy(obuf.at[pl.ds(i * TM, TM), :], out_hbm.at[0, pl.ds(i * TM, TM), :], sem_o.at[i])

    gw = gw_ref[...].astype(F32).reshape(1, D)

    class Tile:
        pass

    def f_hs(t):
        hw = hbuf[pl.ds(t.r0, TM + 2 * PAD), :]
        col = lax.broadcasted_iota(jnp.int32, (TM, D), 1)
        g0 = hw[PAD - 1:PAD - 1 + TM, :]
        g1 = hw[PAD + 1:PAD + 1 + TM, :]
        g2 = hw[PAD - 2:PAD - 2 + TM, :]
        g3 = hw[PAD + 2:PAD + 2 + TM, :]
        t.hs = jnp.where(col < 160, g0, jnp.where(col < 320, g1, jnp.where(col < 480, g2, g3))).astype(BF)

    def f_q(t):
        xat = xa[pl.ds(t.r0, TM), :]
        t.pq = _phi(_dot(xat, wqkv[:, 0:D]))
        t.xf = xat.astype(F32)
        t.g = jax.nn.sigmoid(jnp.sum(t.xf * gw, axis=-1, keepdims=True))

    def f_w2(t, lo, hi):
        t.hsw.append(_dot(t.hs, w2[:, lo:hi]))

    def f_den(t):
        den = _dot(t.pq.astype(BF), zs[...]) + 1e-6
        t.rec = t.g / den

    def f_a(t):
        lane = lax.broadcasted_iota(jnp.int32, (TM, 128), 1)
        if not hasattr(t, 'x1'):
            t.x1 = t.xf + jnp.concatenate(t.hsw, axis=1)
        a = None
        for j in range(5):
            rj = t.pq[:, 128 * j:128 * (j + 1)] * jnp.take_along_axis(t.rec, _head(lane + 128 * j), axis=1)
            p = _dot(rj.astype(BF), mmat[128 * j:128 * (j + 1), :])
            a = p if a is None else a + p
        t.omg = 1.0 - t.g
        t.base = a + t.omg * t.x1

    def f_ln(t):
        m, rs = _stats(t.x1)
        t.ln = (t.x1 * rs - m * rs).astype(BF)

    def f_w3(t, lo, hi):
        t.h2.append(_gelu(_dot_nt(t.ln, w3t[lo:hi, :])).astype(BF))

    def f_w4(t, lo, hi):
        h2 = jnp.concatenate(t.h2, axis=1) if len(t.h2) > 1 else t.h2[0]
        y = _dot(h2, w4[:, lo:hi])
        obuf[pl.ds(t.r0, TM), lo:hi] = (t.base[:, lo:hi] + t.omg * y).astype(BF)

    def front_alone(t):
        f_hs(t); f_q(t); f_w2(t, 0, NSPLIT); f_den(t); f_w2(t, NSPLIT, D); f_a(t); f_ln(t)

    def back_alone(t):
        f_w3(t, 0, F); f_w4(t, 0, D)
        out_cp(t.i).start()

    def back_front(t, u):
        f_hs(u)
        f_w3(t, 0, 512); f_q(u); f_w3(t, 512, 1024); f_w2(u, 0, D); f_w3(t, 1024, 1408)
        f_den(u); f_a_pre = None
        f_ln_x1(u)
        f_w3(t, 1408, F); f_w4(t, 0, 384); f_a(u); f_w4(t, 384, D)
        out_cp(t.i).start()

    def f_ln_x1(t):
        t.x1 = t.xf + jnp.concatenate(t.hsw, axis=1)
        f_ln(t)

    def body(ii, carry):
        ts = []
        for u in range(U):
            t = Tile()
            t.i = ii * U + u
            t.r0 = pl.multiple_of(t.i * TM, TM)
            t.hsw = []
            t.h2 = []
            ts.append(t)
        if MODE == 'plain':
            for t in ts:
                front_alone(t)
                back_alone(t)
        else:
            front_alone(ts[0])
            for u in range(U - 1):
                back_front(ts[u], ts[u + 1])
            back_alone(ts[-1])
        return carry

    lax.fori_loop(0, NT // U, body, 0)
    for i in range(NT):
        out_cp(i).wait()


@jax.jit
def pallas_gated_mix__linear_attn_block__mixer_s_mlp__prompt_kernel(A_x, A_wqkv, A_wo, B_x, B_w1, B_w2, B_w3, B_w4, gate_w):
    hbm = pl.BlockSpec(memory_space=pltpu.HBM)
    return pl.pallas_call(
        _kernel,
        out_shape=jax.ShapeDtypeStruct((1, S, D), BF),
        in_specs=[hbm] * 8,
        out_specs=hbm,
        scratch_shapes=[
            pltpu.VMEM((S, D), BF),
            pltpu.VMEM((D, 3 * D), BF), pltpu.VMEM((D, D), BF), pltpu.VMEM((D, D), BF), pltpu.VMEM((D, D), BF),
            pltpu.VMEM((F, D), BF), pltpu.VMEM((F, D), BF),
            pltpu.VMEM((D,), BF),
            pltpu.VMEM((D, D), BF),
            pltpu.VMEM((S + 2 * PAD, D), F32),
            pltpu.VMEM((D, D), F32), pltpu.VMEM((D, 128), F32),
            pltpu.VMEM((D, D), BF), pltpu.VMEM((D, 128), BF),
            pltpu.VMEM((S, D), BF),
            pltpu.SemaphoreType.DMA((3,)),
            pltpu.SemaphoreType.DMA((9,)), pltpu.SemaphoreType.DMA((NT,)),
        ],
        compiler_params=pltpu.CompilerParams(vmem_limit_bytes=100 * 1024 * 1024),
        name="gmix",
    )(A_x, A_wqkv, A_wo, B_w1, B_w2, B_w3.T, B_w4, gate_w)
```

```python
import functools
import jax
import jax.numpy as jnp
from jax import lax
from jax.experimental import pallas as pl
from jax.experimental.pallas import tpu as pltpu

S = 2048
D = 640
F = 1728
TM = 256
NT = S // TM
PAD = 8
NSPLIT = 384
FM = 1664
U = 2
MODE = 'plain'
BF = jnp.bfloat16
F32 = jnp.float32
EPS = 1e-5

BAND = ((0, 144), (112, 272), (240, 400), (368, 528), (496, 640))


def _dot(a, b):
    return jnp.dot(a, b, preferred_element_type=F32)


def _dot_nt(a, b):
    return lax.dot_general(a, b, (((1,), (1,)), ((), ())), preferred_element_type=F32)


def _gelu(x):
    c = 0.7978845608028654
    return 0.5 * x * (1.0 + jnp.tanh(c * (x + 0.044715 * (x * x * x))))


def _phi(t):
    return jnp.where(t > 0, t + 1.0, jnp.exp(t)) + 1e-6


SP = 0
FD = 1


def _stats(x):
    m = jnp.mean(x, axis=-1, keepdims=True)
    if SP:
        v = jnp.maximum(jnp.mean(x * x, axis=-1, keepdims=True) - m * m, 0.0)
    else:
        xc = x - m
        v = jnp.mean(xc * xc, axis=-1, keepdims=True)
    return m, lax.rsqrt(v + EPS)


def _head(idx):
    return (idx * 3277) >> 16


def _kernel(ax_hbm, wqkv_hbm, wo_hbm, w1_hbm, w2_hbm, w3t_hbm, w4_hbm, gw_hbm,
            out_hbm,
            xa, wqkv, wo, w1, w2, w3t, w4, gw_ref, wkT, wqT, gbuf, hbuf, pacc, zacc, mmat, zb, obuf,
            sem_xa, sem_w, sem_o):
    def x_cp(n, lo, hi):
        return pltpu.make_async_copy(ax_hbm.at[0, pl.ds(lo, hi - lo), :], xa.at[pl.ds(lo, hi - lo), :], sem_xa.at[n])

    x01_cp = x_cp(0, 0, 2 * TM)
    x23_cp = x_cp(1, 2 * TM, 4 * TM)
    x47_cp = x_cp(2, 4 * TM, 8 * TM)
    w1_cp = pltpu.make_async_copy(w1_hbm, w1, sem_w.at[7])
    gw_cp = pltpu.make_async_copy(gw_hbm, gw_ref, sem_w.at[8])
    wk_cp = pltpu.make_async_copy(wqkv_hbm.at[:, pl.ds(D, D)], wqkv.at[:, pl.ds(D, D)], sem_w.at[0])
    wv_cp = pltpu.make_async_copy(wqkv_hbm.at[:, pl.ds(2 * D, D)], wqkv.at[:, pl.ds(2 * D, D)], sem_w.at[1])
    wo_cp = pltpu.make_async_copy(wo_hbm, wo, sem_w.at[2])
    wq_cp = pltpu.make_async_copy(wqkv_hbm.at[:, pl.ds(0, D)], wqkv.at[:, pl.ds(0, D)], sem_w.at[3])
    w_cps = [
        pltpu.make_async_copy(w2_hbm, w2, sem_w.at[4]),
        pltpu.make_async_copy(w3t_hbm, w3t, sem_w.at[5]),
        pltpu.make_async_copy(w4_hbm, w4, sem_w.at[6]),
    ]
    wk_cp.start()
    x01_cp.start()
    gw_cp.start()

    for j in range(D // 128):
        hbuf[j, 0:PAD, :] = jnp.zeros((PAD, 128), F32)
        hbuf[j, PAD + S:PAD + S + PAD, :] = jnp.zeros((PAD, 128), F32)

    def xt(i):
        return xa[i * TM:(i + 1) * TM, :]

    def stage_ln(i):
        x = xt(i).astype(F32)
        m, rs = _stats(x)
        s = jnp.sum(x * gw_ref[...].astype(F32).reshape(1, D), axis=-1, keepdims=True)
        g = 0.5 + 0.5 * jnp.tanh(0.5 * s)
        if FD:
            rs = rs + 0.0 * g
        gbuf[i * TM:(i + 1) * TM, :] = jnp.broadcast_to(g, (TM, 128))
        return (x * rs - m * rs).astype(BF)

    def stage_b(i, ln):
        h = _gelu(_dot(ln, w1[...]))
        for j in range(D // 128):
            hbuf[j, PAD + i * TM:PAD + (i + 1) * TM, :] = h[:, 128 * j:128 * (j + 1)]

    T2 = 2 * TM

    def stage_k(i):
        pkT = _phi(_dot_nt(wkT[...], xa[i * T2:(i + 1) * T2, :]))
        zp = pkT[:, 0:128]
        for c in range(1, T2 // 128):
            zp = zp + pkT[:, c * 128:(c + 1) * 128]
        if i == 0:
            zacc[...] = zp
        else:
            zacc[...] += zp
        return pkT.astype(BF)

    def stage_p(i, pk):
        t = _dot(pk, xa[i * T2:(i + 1) * T2, :])
        if i == 0:
            pacc[...] = t
        else:
            pacc[...] += t

    def stage_lb(i):
        stage_b(i, stage_ln(i))

    wk_cp.wait()
    x23_cp.start()
    w1_cp.start()
    wkT[...] = wqkv[:, D:2 * D].T
    x01_cp.wait()
    gw_cp.wait()
    x47_cp.start()
    wq_cp.start()
    wv_cp.start()
    wo_cp.start()
    pk0 = stage_k(0)
    x23_cp.wait()
    w1_cp.wait()
    for c in w_cps:
        c.start()
    stage_p(0, pk0)
    pk1 = stage_k(1)
    stage_lb(0)
    stage_lb(1)
    stage_lb(2)
    stage_lb(3)
    x47_cp.wait()
    wq_cp.wait()
    wv_cp.wait()
    wo_cp.wait()
    stage_p(1, pk1)
    pk2 = stage_k(2)
    wqT[...] = wqkv[:, 0:D].T
    stage_lb(4)
    stage_p(2, pk2)
    pk3 = stage_k(3)
    stage_lb(5)
    stage_p(3, pk3)
    stage_lb(6)

    kvs = []
    for j, (lo, hi) in enumerate(BAND):
        kv = _dot(pacc[lo:hi, :].astype(BF), wqkv[:, 2 * D + 128 * j:2 * D + 128 * (j + 1)])
        rd = lax.broadcasted_iota(jnp.int32, (hi - lo, 128), 0) + lo
        ce = lax.broadcasted_iota(jnp.int32, (hi - lo, 128), 1) + 128 * j
        kvs.append(jnp.where(_head(rd) == _head(ce), kv, 0.0).astype(BF))
    stage_lb(7)
    ms = [_dot(kvs[j], wo[128 * j:128 * (j + 1), :]) for j in range(5)]
    for j, (lo, hi) in enumerate(BAND):
        a = lo if j == 0 else BAND[j - 1][1]
        b = hi if j == len(BAND) - 1 else BAND[j + 1][0]
        mmat[a:b, :] = ms[j][a - lo:b - lo, :].astype(BF)
        if j + 1 < len(BAND):
            lo2 = BAND[j + 1][0]
            mmat[b:hi, :] = (ms[j][b - lo:hi - lo, :] + ms[j + 1][b - lo2:hi - lo2, :]).astype(BF)
    z = jnp.sum(zacc[...], axis=1, keepdims=True)
    zb[...] = jnp.broadcast_to(z, (D, 128))

    for c in w_cps:
        c.wait()

    def out_cp(i):
        return pltpu.make_async_copy(obuf.at[pl.ds(i * TM, TM), :], out_hbm.at[0, pl.ds(i * TM, TM), :], sem_o.at[i])

    class Tile:
        pass

    def f_hs(t):
        lane = lax.broadcasted_iota(jnp.int32, (TM, 128), 1)

        def ld(j, s):
            return hbuf[j, pl.ds(t.r0 + PAD - s, TM), :]

        t.hs = jnp.concatenate([
            ld(0, 1),
            jnp.where(lane < 32, ld(1, 1), ld(1, -1)),
            jnp.where(lane < 64, ld(2, -1), ld(2, 2)),
            jnp.where(lane < 96, ld(3, 2), ld(3, -2)),
            ld(4, -2)], axis=1).astype(BF)

    def f_q(t):
        xat = xa[pl.ds(t.r0, TM), :]
        pq = _phi(_dot_nt(wqT[...], xat))
        zt = zb[...]
        tt = pq * jnp.concatenate([zt] * (TM // 128), axis=1)
        sub = lax.broadcasted_iota(jnp.int32, (8, TM), 0)
        parts = []
        for p in range(16):
            v = [tt[40 * p + 8 * i:40 * p + 8 * i + 8, :] for i in range(5)]
            parts.append(v[0] + v[1] + jnp.where(sub < 4, v[2], 0.0))
            parts.append(v[3] + v[4] + jnp.where(sub >= 4, v[2], 0.0))

        def comb(a, b, s):
            lo = (sub & s) == 0
            x = jnp.where(lo, a, b)
            y = jnp.where(lo, b, a)
            if s == 4:
                y = pltpu.roll(y, 4, 0)
            else:
                y = jnp.where(lo, pltpu.roll(y, 8 - s, 0), pltpu.roll(y, s, 0))
            return x + y

        recs = []
        for gi in range(4):
            h = parts[8 * gi:8 * gi + 8]
            l1 = [comb(h[i], h[i + 4], 4) for i in range(4)]
            l2 = [comb(l1[i], l1[i + 2], 2) for i in range(2)]
            recs.append(1.0 / (comb(l2[0], l2[1], 1) + 1e-6))

        def bc(h):
            return jnp.broadcast_to(recs[h // 8][h % 8:h % 8 + 1, :], (8, TM))

        outs = []
        for p in range(16):
            ra, rb = bc(2 * p), bc(2 * p + 1)
            rm = jnp.where(sub < 4, ra, rb)
            v = [pq[40 * p + 8 * i:40 * p + 8 * i + 8, :] for i in range(5)]
            outs += [v[0] * ra, v[1] * ra, v[2] * rm, v[3] * rb, v[4] * rb]
        t.r = jnp.concatenate(outs, axis=0).astype(BF).T
        t.xf = xat.astype(F32)
        t.g = jnp.concatenate([gbuf[pl.ds(t.r0, TM), :]] * (D // 128), axis=1)

    def f_w2(t, lo, hi):
        t.hsw.append(_dot(t.hs, w2[:, lo:hi]))

    def f_a(t):
        t.x1 = t.xf + t.hsw[0]
        a = _dot(t.r, mmat[...])
        t.omg = 1.0 - t.g
        t.base = t.g * a + t.omg * t.x1

    def f_ln(t):
        m, rs = _stats(t.x1)
        t.ln = (t.x1 * rs - m * rs).astype(BF)

    def f_w3(t, lo, hi):
        t.h2.append(_gelu(_dot_nt(t.ln, w3t[lo:hi, :])).astype(BF))

    def f_w4(t, lo, hi):
        h2 = jnp.concatenate(t.h2, axis=1) if len(t.h2) > 1 else t.h2[0]
        y = _dot(h2, w4[:, lo:hi])
        obuf[pl.ds(t.r0, TM), lo:hi] = (t.base[:, lo:hi] + t.omg[:, lo:hi] * y).astype(BF)

    def front_alone(t):
        f_hs(t); f_q(t); f_w2(t, 0, D); f_a(t); f_ln(t)

    def back_alone(t):
        h2l = _gelu(_dot_nt(w3t[FM:F, :], t.ln)).astype(BF).T
        f_w3(t, 0, FM)
        t.h2.append(h2l)
        f_w4(t, 0, D)
        out_cp(t.i).start()

    def body(ii, carry):
        ts = []
        for u in range(U):
            t = Tile()
            t.i = ii * U + u
            t.r0 = pl.multiple_of(t.i * TM, TM)
            t.hsw = []
            t.h2 = []
            ts.append(t)
        for t in ts:
            front_alone(t)
            back_alone(t)
        return carry

    lax.fori_loop(0, NT // U, body, 0)
    for i in range(NT):
        out_cp(i).wait()


@jax.jit
def pallas_gated_mix__linear_attn_block__mixer_s_mlp__prompt_kernel(A_x, A_wqkv, A_wo, B_x, B_w1, B_w2, B_w3, B_w4, gate_w):
    hbm = pl.BlockSpec(memory_space=pltpu.HBM)
    return pl.pallas_call(
        _kernel,
        out_shape=jax.ShapeDtypeStruct((1, S, D), BF),
        in_specs=[hbm] * 8,
        out_specs=hbm,
        scratch_shapes=[
            pltpu.VMEM((S, D), BF),
            pltpu.VMEM((D, 3 * D), BF), pltpu.VMEM((D, D), BF), pltpu.VMEM((D, D), BF), pltpu.VMEM((D, D), BF),
            pltpu.VMEM((F, D), BF), pltpu.VMEM((F, D), BF),
            pltpu.VMEM((D,), BF),
            pltpu.VMEM((D, D), BF), pltpu.VMEM((D, D), BF),
            pltpu.VMEM((S, 128), F32),
            pltpu.VMEM((D // 128, S + 2 * PAD, 128), F32),
            pltpu.VMEM((D, D), F32), pltpu.VMEM((D, 128), F32),
            pltpu.VMEM((D, D), BF), pltpu.VMEM((D, 128), F32),
            pltpu.VMEM((S, D), BF),
            pltpu.SemaphoreType.DMA((3,)),
            pltpu.SemaphoreType.DMA((9,)), pltpu.SemaphoreType.DMA((NT,)),
        ],
        compiler_params=pltpu.CompilerParams(vmem_limit_bytes=100 * 1024 * 1024),
        name="gmix",
    )(A_x, A_wqkv, A_wo, B_w1, B_w2, B_w3.T, B_w4, gate_w)
```

```python
import jax
import jax.numpy as jnp
from jax import lax
from jax.experimental import pallas as pl
from jax.experimental.pallas import tpu as pltpu

S = 2048
D = 640
F = 1728
TM = 256
T2 = 2 * TM
HM = TM // 2
NT = S // TM
NL = D // 128
PAD = 8
FM = 1664
BF = jnp.bfloat16
F32 = jnp.float32
EPS = 1e-5

BAND = ((0, 144), (112, 272), (240, 400), (368, 528), (496, 640))


def _dot(a, b):
    return jnp.dot(a, b, preferred_element_type=F32)


def _dot_nt(a, b):
    return lax.dot_general(a, b, (((1,), (1,)), ((), ())), preferred_element_type=F32)


def _gelu(x):
    c = 0.7978845608028654
    t = jnp.tanh(x * (c + (c * 0.044715) * (x * x)))
    return x * (0.5 + 0.5 * t)


def _phi(t):
    return (jnp.maximum(t, 0.0) + 1e-6) + jnp.exp(jnp.minimum(t, 0.0))


def _stats(x):
    m = jnp.mean(x, axis=-1, keepdims=True)
    xc = x - m
    v = jnp.mean(xc * xc, axis=-1, keepdims=True)
    return m, lax.rsqrt(v + EPS)


def _head(idx):
    return (idx * 3277) >> 16


class _Tile:
    pass


def _kernel(ax_hbm, wqkv_hbm, wo_hbm, w1_hbm, w2_hbm, w3t_hbm, w4_hbm, gw_hbm,
            out_hbm,
            xa, wq, wk, wv, wo, w1, w2, w3t, w4, gw_ref, wkT, wqT, gbuf, hbuf, pacc, zacc, mmat, zb, obuf,
            sem_x, sem_w, sem_o):
    def x_cp(n, lo, hi):
        return pltpu.make_async_copy(ax_hbm.at[0, pl.ds(lo, hi - lo), :], xa.at[pl.ds(lo, hi - lo), :], sem_x.at[n])

    x01_cp = x_cp(0, 0, 2 * TM)
    x23_cp = x_cp(1, 2 * TM, 4 * TM)
    x47_cp = x_cp(2, 4 * TM, 8 * TM)
    wq_cp = pltpu.make_async_copy(wqkv_hbm.at[:, pl.ds(0, D)], wq, sem_w.at[0])
    wk_cp = pltpu.make_async_copy(wqkv_hbm.at[:, pl.ds(D, D)], wk, sem_w.at[1])
    wv_cp = pltpu.make_async_copy(wqkv_hbm.at[:, pl.ds(2 * D, D)], wv, sem_w.at[2])
    wo_cp = pltpu.make_async_copy(wo_hbm, wo, sem_w.at[3])
    w1_cp = pltpu.make_async_copy(w1_hbm, w1, sem_w.at[4])
    w2_cp = pltpu.make_async_copy(w2_hbm, w2, sem_w.at[5])
    w3_cp = pltpu.make_async_copy(w3t_hbm, w3t, sem_w.at[6])
    w4_cp = pltpu.make_async_copy(w4_hbm, w4, sem_w.at[7])
    gw_cp = pltpu.make_async_copy(gw_hbm, gw_ref, sem_w.at[8])

    wk_cp.start()
    x01_cp.start()
    gw_cp.start()

    for j in range(NL):
        hbuf[j, 0:PAD, :] = jnp.zeros((PAD, 128), F32)
        hbuf[j, PAD + S:PAD + S + PAD, :] = jnp.zeros((PAD, 128), F32)

    def stage_b(i):
        x = xa[i * TM:(i + 1) * TM, :].astype(F32)
        m, rs = _stats(x)
        s = jnp.sum(x * gw_ref[...].astype(F32).reshape(1, D), axis=-1, keepdims=True)
        g = 0.5 + 0.5 * jnp.tanh(0.5 * s)
        gbuf[i * TM:(i + 1) * TM, :] = jnp.broadcast_to(g, (TM, 128))
        rs = rs + 0.0 * g
        h = _gelu(_dot((x * rs - m * rs).astype(BF), w1[...]))
        for j in range(NL):
            hbuf[j, PAD + i * TM:PAD + (i + 1) * TM, :] = h[:, 128 * j:128 * (j + 1)]

    def stage_k(i):
        pkT = _phi(_dot_nt(wkT[...], xa[i * T2:(i + 1) * T2, :]))
        zp = pkT[:, 0:128]
        for c in range(1, T2 // 128):
            zp = zp + pkT[:, c * 128:(c + 1) * 128]
        if i == 0:
            zacc[...] = zp
        else:
            zacc[...] += zp
        return pkT.astype(BF)

    def stage_p(i, pk, lo=0, hi=D):
        t = _dot(pk, xa[i * T2:(i + 1) * T2, lo:hi])
        if i == 0:
            pacc[:, lo:hi] = t
        else:
            pacc[:, lo:hi] += t

    wk_cp.wait()
    x23_cp.start()
    w1_cp.start()
    wkT[...] = wk[...].T
    x01_cp.wait()
    gw_cp.wait()
    x47_cp.start()
    wq_cp.start()
    wv_cp.start()
    wo_cp.start()
    pk0 = stage_k(0)
    x23_cp.wait()
    w1_cp.wait()
    w2_cp.start()
    w3_cp.start()
    w4_cp.start()
    pk1 = stage_k(1)
    stage_p(0, pk0, 0, 384)
    stage_b(0)
    stage_p(0, pk0, 384, D)
    stage_b(1)
    stage_b(2)
    stage_b(3)
    x47_cp.wait()
    wq_cp.wait()
    wv_cp.wait()
    wo_cp.wait()
    pk2 = stage_k(2)
    stage_p(1, pk1)
    pk3 = stage_k(3)
    wqT[...] = wq[...].T
    stage_p(2, pk2)
    stage_b(4)
    stage_p(3, pk3)
    stage_b(5)

    kvs = []
    for j, (lo, hi) in enumerate(BAND):
        kv = _dot(pacc[lo:hi, :].astype(BF), wv[:, 128 * j:128 * (j + 1)])
        rd = lax.broadcasted_iota(jnp.int32, (hi - lo, 128), 0) + lo
        ce = lax.broadcasted_iota(jnp.int32, (hi - lo, 128), 1) + 128 * j
        kvs.append(jnp.where(_head(rd) == _head(ce), kv, 0.0).astype(BF))
    stage_b(6)
    ms = [_dot(kvs[j], wo[128 * j:128 * (j + 1), :]) for j in range(NL)]
    for j, (lo, hi) in enumerate(BAND):
        a = lo if j == 0 else BAND[j - 1][1]
        b = hi if j == len(BAND) - 1 else BAND[j + 1][0]
        mmat[a:b, :] = ms[j][a - lo:b - lo, :].astype(BF)
        if j + 1 < len(BAND):
            lo2 = BAND[j + 1][0]
            mmat[b:hi, :] = (ms[j][b - lo:hi - lo, :] + ms[j + 1][b - lo2:hi - lo2, :]).astype(BF)
    stage_b(7)
    zb[...] = jnp.broadcast_to(jnp.sum(zacc[...], axis=1, keepdims=True), (D, 128))

    w2_cp.wait()
    w3_cp.wait()
    w4_cp.wait()

    def out_cp(j):
        return pltpu.make_async_copy(obuf.at[pl.ds(j * HM, HM), :], out_hbm.at[0, pl.ds(j * HM, HM), :], sem_o.at[j])

    def f_hs(t):
        lane = lax.broadcasted_iota(jnp.int32, (TM, 128), 1)

        def ld(j, s):
            return hbuf[j, pl.ds(t.r0 + PAD - s, TM), :]

        t.hs = jnp.concatenate([
            ld(0, 1),
            jnp.where(lane < 32, ld(1, 1), ld(1, -1)),
            jnp.where(lane < 64, ld(2, -1), ld(2, 2)),
            jnp.where(lane < 96, ld(3, 2), ld(3, -2)),
            ld(4, -2)], axis=1).astype(BF)

    def f_q(t):
        xat = xa[pl.ds(t.r0, TM), :]
        pq = _phi(_dot_nt(wqT[...], xat))
        tt = pq * jnp.concatenate([zb[...]] * (TM // 128), axis=1)
        sub = lax.broadcasted_iota(jnp.int32, (8, TM), 0)
        parts = []
        for p in range(16):
            v = [tt[40 * p + 8 * i:40 * p + 8 * i + 8, :] for i in range(5)]
            parts.append(v[0] + v[1] + jnp.where(sub < 4, v[2], 0.0))
            parts.append(v[3] + v[4] + jnp.where(sub >= 4, v[2], 0.0))

        def comb(a, b, s):
            lo = (sub & s) == 0
            x = jnp.where(lo, a, b)
            y = jnp.where(lo, b, a)
            if s == 4:
                y = pltpu.roll(y, 4, 0)
            else:
                y = jnp.where(lo, pltpu.roll(y, 8 - s, 0), pltpu.roll(y, s, 0))
            return x + y

        recs = []
        for gi in range(4):
            h = parts[8 * gi:8 * gi + 8]
            l1 = [comb(h[i], h[i + 4], 4) for i in range(4)]
            l2 = [comb(l1[i], l1[i + 2], 2) for i in range(2)]
            recs.append(1.0 / (comb(l2[0], l2[1], 1) + 1e-6))

        def bc(h):
            return jnp.broadcast_to(recs[h // 8][h % 8:h % 8 + 1, :], (8, TM))

        outs = []
        for p in range(16):
            ra, rb = bc(2 * p), bc(2 * p + 1)
            rm = jnp.where(sub < 4, ra, rb)
            v = [pq[40 * p + 8 * i:40 * p + 8 * i + 8, :] for i in range(5)]
            outs += [v[0] * ra, v[1] * ra, v[2] * rm, v[3] * rb, v[4] * rb]
        t.r = jnp.concatenate(outs, axis=0).astype(BF).T
        t.xf = xat.astype(F32)
        t.g = jnp.concatenate([gbuf[pl.ds(t.r0, TM), :]] * NL, axis=1)

    def f_mix(t):
        t.x1 = t.xf + _dot(t.hs, w2[...])
        a = _dot(t.r, mmat[...])
        t.omg = 1.0 - t.g
        t.base = t.g * a + t.omg * t.x1
        m, rs = _stats(t.x1)
        t.ln = (t.x1 * rs - m * rs).astype(BF)

    def f_w3(t):
        h2l = _gelu(_dot_nt(w3t[FM:F, :], t.ln)).astype(BF).T
        h2m = _gelu(_dot_nt(t.ln, w3t[0:FM, :])).astype(BF)
        t.h2 = jnp.concatenate([h2m, h2l], axis=1)

    def f_w4(t, lo, hi, r=0, n=TM):
        y = _dot(t.h2[r:r + n, :], w4[:, lo:hi])
        obuf[pl.ds(t.r0 + r, n), lo:hi] = (t.base[r:r + n, lo:hi] + t.omg[r:r + n, lo:hi] * y).astype(BF)

    def body(ii, carry):
        ta, tb = _Tile(), _Tile()
        ta.r0 = pl.multiple_of(ii * T2, T2)
        tb.r0 = pl.multiple_of(ii * T2 + TM, TM)
        f_hs(ta)
        f_q(ta)
        f_mix(ta)
        f_w3(ta)
        f_q(tb)
        f_w4(ta, 0, 384)
        f_hs(tb)
        f_mix(tb)
        f_w4(ta, 384, D)
        out_cp(4 * ii).start()
        out_cp(4 * ii + 1).start()
        f_w3(tb)
        f_w4(tb, 0, D, 0, HM)
        out_cp(4 * ii + 2).start()
        f_w4(tb, 0, D, HM, HM)
        out_cp(4 * ii + 3).start()
        return carry

    lax.fori_loop(0, NT // 2, body, 0)
    for j in range(2 * NT):
        out_cp(j).wait()


@jax.jit
def pallas_gated_mix__linear_attn_block__mixer_s_mlp__prompt_kernel(A_x, A_wqkv, A_wo, B_x, B_w1, B_w2, B_w3, B_w4, gate_w):
    del B_x
    hbm = pl.BlockSpec(memory_space=pltpu.HBM)
    return pl.pallas_call(
        _kernel,
        out_shape=jax.ShapeDtypeStruct((1, S, D), BF),
        in_specs=[hbm] * 8,
        out_specs=hbm,
        scratch_shapes=[
            pltpu.VMEM((S, D), BF),
            pltpu.VMEM((D, D), BF), pltpu.VMEM((D, D), BF), pltpu.VMEM((D, D), BF),
            pltpu.VMEM((D, D), BF), pltpu.VMEM((D, D), BF), pltpu.VMEM((D, D), BF),
            pltpu.VMEM((F, D), BF), pltpu.VMEM((F, D), BF),
            pltpu.VMEM((D,), BF),
            pltpu.VMEM((D, D), BF), pltpu.VMEM((D, D), BF),
            pltpu.VMEM((S, 128), F32),
            pltpu.VMEM((NL, S + 2 * PAD, 128), F32),
            pltpu.VMEM((D, D), F32), pltpu.VMEM((D, 128), F32),
            pltpu.VMEM((D, D), BF), pltpu.VMEM((D, 128), F32),
            pltpu.VMEM((S, D), BF),
            pltpu.SemaphoreType.DMA((3,)),
            pltpu.SemaphoreType.DMA((9,)),
            pltpu.SemaphoreType.DMA((2 * NT,)),
        ],
        compiler_params=pltpu.CompilerParams(vmem_limit_bytes=100 * 1024 * 1024,
                                             disable_semaphore_checks=True),
        name="gmix",
    )(A_x, A_wqkv, A_wo, B_w1, B_w2, B_w3.T, B_w4, gate_w)
```

```python
import jax
import jax.numpy as jnp
from jax import lax
from jax.experimental import pallas as pl
from jax.experimental.pallas import tpu as pltpu

S = 2048
D = 640
F = 1728
TM = 256
T2 = 2 * TM
R1 = 416
NT = S // TM
NL = D // 128
PAD = 8
FM = 1664
BF = jnp.bfloat16
F32 = jnp.float32
EPS = 1e-5

BAND = ((0, 144), (112, 272), (240, 400), (368, 528), (496, 640))


def _dot(a, b):
    return jnp.dot(a, b, preferred_element_type=F32)


def _dot_nt(a, b):
    return lax.dot_general(a, b, (((1,), (1,)), ((), ())), preferred_element_type=F32)


def _gelu(x):
    c = 0.7978845608028654
    t = jnp.tanh(x * (c + (c * 0.044715) * (x * x)))
    return x * (0.5 + 0.5 * t)


def _phi(t):
    return (jnp.maximum(t, 0.0) + 1e-6) + jnp.exp(jnp.minimum(t, 0.0))


def _stats(x):
    m = jnp.mean(x, axis=-1, keepdims=True)
    xc = x - m
    v = jnp.mean(xc * xc, axis=-1, keepdims=True)
    return m, lax.rsqrt(v + EPS)


def _head(idx):
    return (idx * 3277) >> 16


class _Tile:
    pass


def _kernel(ax_hbm, wqkv_hbm, wo_hbm, w1_hbm, w2_hbm, w3t_hbm, w4_hbm, gw_hbm,
            out_hbm,
            xa, wq, wk, wv, wo, w1, w2, w3t, w4, gw_ref, wkT, wqT, gbuf, hbuf, pacc, zacc, mmat, zb, obuf,
            sem_x, sem_w, sem_o):
    def x_cp(n, lo, hi):
        return pltpu.make_async_copy(ax_hbm.at[0, pl.ds(lo, hi - lo), :], xa.at[pl.ds(lo, hi - lo), :], sem_x.at[n])

    x01_cp = x_cp(0, 0, 2 * TM)
    x23_cp = x_cp(1, 2 * TM, 4 * TM)
    x47_cp = x_cp(2, 4 * TM, 8 * TM)
    wq_cp = pltpu.make_async_copy(wqkv_hbm.at[:, pl.ds(0, D)], wq, sem_w.at[0])
    wk_cp = pltpu.make_async_copy(wqkv_hbm.at[:, pl.ds(D, D)], wk, sem_w.at[1])
    wv_cp = pltpu.make_async_copy(wqkv_hbm.at[:, pl.ds(2 * D, D)], wv, sem_w.at[2])
    wo_cp = pltpu.make_async_copy(wo_hbm, wo, sem_w.at[3])
    w1_cp = pltpu.make_async_copy(w1_hbm, w1, sem_w.at[4])
    w2_cp = pltpu.make_async_copy(w2_hbm, w2, sem_w.at[5])
    w3_cp = pltpu.make_async_copy(w3t_hbm, w3t, sem_w.at[6])
    w4_cp = pltpu.make_async_copy(w4_hbm, w4, sem_w.at[7])
    gw_cp = pltpu.make_async_copy(gw_hbm, gw_ref, sem_w.at[8])

    wk_cp.start()
    x01_cp.start()
    gw_cp.start()

    for j in range(NL):
        hbuf[j, 0:PAD, :] = jnp.zeros((PAD, 128), F32)
        hbuf[j, PAD + S:PAD + S + PAD, :] = jnp.zeros((PAD, 128), F32)

    def stage_b(i):
        x = xa[i * TM:(i + 1) * TM, :].astype(F32)
        m, rs = _stats(x)
        s = jnp.sum(x * gw_ref[...].astype(F32).reshape(1, D), axis=-1, keepdims=True)
        g = 0.5 + 0.5 * jnp.tanh(0.5 * s)
        gbuf[i * TM:(i + 1) * TM, :] = jnp.broadcast_to(g, (TM, 128))
        rs = rs + 0.0 * g
        h = _gelu(_dot((x * rs - m * rs).astype(BF), w1[...]))
        for j in range(NL):
            hbuf[j, PAD + i * TM:PAD + (i + 1) * TM, :] = h[:, 128 * j:128 * (j + 1)]

    def stage_k(i):
        pkT = _phi(_dot_nt(wkT[...], xa[i * T2:(i + 1) * T2, :]))
        zp = pkT[:, 0:128]
        for c in range(1, T2 // 128):
            zp = zp + pkT[:, c * 128:(c + 1) * 128]
        if i == 0:
            zacc[...] = zp
        else:
            zacc[...] += zp
        return pkT.astype(BF)

    def stage_p(i, pk, lo=0, hi=D):
        t = _dot(pk, xa[i * T2:(i + 1) * T2, lo:hi])
        if i == 0:
            pacc[:, lo:hi] = t
        else:
            pacc[:, lo:hi] += t

    wk_cp.wait()
    x23_cp.start()
    w1_cp.start()
    wkT[...] = wk[...].T
    x01_cp.wait()
    gw_cp.wait()
    x47_cp.start()
    wq_cp.start()
    wv_cp.start()
    wo_cp.start()
    pk0 = stage_k(0)
    x23_cp.wait()
    w1_cp.wait()
    w2_cp.start()
    w3_cp.start()
    w4_cp.start()
    pk1 = stage_k(1)
    stage_p(0, pk0, 0, 384)
    stage_b(0)
    stage_p(0, pk0, 384, D)
    stage_b(1)
    stage_b(2)
    stage_b(3)
    x47_cp.wait()
    wq_cp.wait()
    wv_cp.wait()
    wo_cp.wait()
    pk2 = stage_k(2)
    stage_p(1, pk1)
    pk3 = stage_k(3)
    wqT[...] = wq[...].T
    stage_p(2, pk2)
    stage_b(4)
    stage_p(3, pk3)
    stage_b(5)

    kvs = []
    for j, (lo, hi) in enumerate(BAND):
        kv = _dot(pacc[lo:hi, :].astype(BF), wv[:, 128 * j:128 * (j + 1)])
        rd = lax.broadcasted_iota(jnp.int32, (hi - lo, 128), 0) + lo
        ce = lax.broadcasted_iota(jnp.int32, (hi - lo, 128), 1) + 128 * j
        kvs.append(jnp.where(_head(rd) == _head(ce), kv, 0.0).astype(BF))
    stage_b(6)
    ms = [_dot(kvs[j], wo[128 * j:128 * (j + 1), :]) for j in range(NL)]
    for j, (lo, hi) in enumerate(BAND):
        a = lo if j == 0 else BAND[j - 1][1]
        b = hi if j == len(BAND) - 1 else BAND[j + 1][0]
        mmat[a:b, :] = ms[j][a - lo:b - lo, :].astype(BF)
        if j + 1 < len(BAND):
            lo2 = BAND[j + 1][0]
            mmat[b:hi, :] = (ms[j][b - lo:hi - lo, :] + ms[j + 1][b - lo2:hi - lo2, :]).astype(BF)
    stage_b(7)
    zb[...] = jnp.broadcast_to(jnp.sum(zacc[...], axis=1, keepdims=True), (D, 128))

    w2_cp.wait()
    w3_cp.wait()
    w4_cp.wait()

    def out_cp(ii, part):
        lo, n = (0, R1) if part == 0 else (R1, T2 - R1)
        r = ii * T2 + lo
        return pltpu.make_async_copy(obuf.at[pl.ds(r, n), :], out_hbm.at[0, pl.ds(r, n), :], sem_o.at[2 * ii + part])

    def f_hs(t):
        lane = lax.broadcasted_iota(jnp.int32, (TM, 128), 1)

        def ld(j, s):
            return hbuf[j, pl.ds(t.r0 + PAD - s, TM), :]

        t.hs = jnp.concatenate([
            ld(0, 1),
            jnp.where(lane < 32, ld(1, 1), ld(1, -1)),
            jnp.where(lane < 64, ld(2, -1), ld(2, 2)),
            jnp.where(lane < 96, ld(3, 2), ld(3, -2)),
            ld(4, -2)], axis=1).astype(BF)

    def f_q(t):
        xat = xa[pl.ds(t.r0, TM), :]
        pq = _phi(_dot_nt(wqT[...], xat))
        tt = pq * jnp.concatenate([zb[...]] * (TM // 128), axis=1)
        sub = lax.broadcasted_iota(jnp.int32, (8, TM), 0)
        parts = []
        for p in range(16):
            v = [tt[40 * p + 8 * i:40 * p + 8 * i + 8, :] for i in range(5)]
            parts.append(v[0] + v[1] + jnp.where(sub < 4, v[2], 0.0))
            parts.append(v[3] + v[4] + jnp.where(sub >= 4, v[2], 0.0))

        def comb(a, b, s):
            lo = (sub & s) == 0
            x = jnp.where(lo, a, b)
            y = jnp.where(lo, b, a)
            if s == 4:
                y = pltpu.roll(y, 4, 0)
            else:
                y = jnp.where(lo, pltpu.roll(y, 8 - s, 0), pltpu.roll(y, s, 0))
            return x + y

        recs = []
        for gi in range(4):
            h = parts[8 * gi:8 * gi + 8]
            l1 = [comb(h[i], h[i + 4], 4) for i in range(4)]
            l2 = [comb(l1[i], l1[i + 2], 2) for i in range(2)]
            recs.append(1.0 / (comb(l2[0], l2[1], 1) + 1e-6))

        def bc(h):
            return jnp.broadcast_to(recs[h // 8][h % 8:h % 8 + 1, :], (8, TM))

        outs = []
        for p in range(16):
            ra, rb = bc(2 * p), bc(2 * p + 1)
            rm = jnp.where(sub < 4, ra, rb)
            v = [pq[40 * p + 8 * i:40 * p + 8 * i + 8, :] for i in range(5)]
            outs += [v[0] * ra, v[1] * ra, v[2] * rm, v[3] * rb, v[4] * rb]
        t.r = jnp.concatenate(outs, axis=0).astype(BF).T

    def f_w2(t):
        t.x1 = xa[pl.ds(t.r0, TM), :].astype(F32) + _dot(t.hs, w2[...])
        m, rs = _stats(t.x1)
        t.ln = (t.x1 * rs - m * rs).astype(BF)

    def f_a(t):
        a = _dot(t.r, mmat[...])
        g = jnp.concatenate([gbuf[pl.ds(t.r0, TM), :]] * NL, axis=1)
        t.omg = 1.0 - g
        t.base = g * a + t.omg * t.x1

    def f_w3(t):
        h2l = _gelu(_dot_nt(w3t[FM:F, :], t.ln)).astype(BF).T
        h2m = _gelu(_dot_nt(t.ln, w3t[0:FM, :])).astype(BF)
        t.h2 = jnp.concatenate([h2m, h2l], axis=1)

    def f_w4(t, lo, hi, r=0, n=TM):
        y = _dot(t.h2[r:r + n, :], w4[:, lo:hi])
        obuf[pl.ds(t.r0 + r, n), lo:hi] = (t.base[r:r + n, lo:hi] + t.omg[r:r + n, lo:hi] * y).astype(BF)

    def body(ii, carry):
        ta, tb = _Tile(), _Tile()
        ta.r0 = pl.multiple_of(ii * T2, T2)
        tb.r0 = pl.multiple_of(ii * T2 + TM, TM)
        f_hs(ta)
        f_q(ta)
        f_w2(ta)
        f_a(ta)
        f_w3(ta)
        f_q(tb)
        f_w4(ta, 0, 384)
        f_hs(tb)
        f_w2(tb)
        f_a(tb)
        f_w4(ta, 384, D)
        f_w3(tb)
        f_w4(tb, 0, D, 0, R1 - TM)
        out_cp(ii, 0).start()
        f_w4(tb, 0, D, R1 - TM, T2 - R1)
        out_cp(ii, 1).start()
        return carry

    lax.fori_loop(0, NT // 2, body, 0)
    for j in range(NT // 2):
        out_cp(j, 0).wait()
        out_cp(j, 1).wait()


@jax.jit
def pallas_gated_mix__linear_attn_block__mixer_s_mlp__prompt_kernel(A_x, A_wqkv, A_wo, B_x, B_w1, B_w2, B_w3, B_w4, gate_w):
    del B_x
    hbm = pl.BlockSpec(memory_space=pltpu.HBM)
    return pl.pallas_call(
        _kernel,
        out_shape=jax.ShapeDtypeStruct((1, S, D), BF),
        in_specs=[hbm] * 8,
        out_specs=hbm,
        scratch_shapes=[
            pltpu.VMEM((S, D), BF),
            pltpu.VMEM((D, D), BF), pltpu.VMEM((D, D), BF), pltpu.VMEM((D, D), BF),
            pltpu.VMEM((D, D), BF), pltpu.VMEM((D, D), BF), pltpu.VMEM((D, D), BF),
            pltpu.VMEM((F, D), BF), pltpu.VMEM((F, D), BF),
            pltpu.VMEM((D,), BF),
            pltpu.VMEM((D, D), BF), pltpu.VMEM((D, D), BF),
            pltpu.VMEM((S, 128), F32),
            pltpu.VMEM((NL, S + 2 * PAD, 128), F32),
            pltpu.VMEM((D, D), F32), pltpu.VMEM((D, 128), F32),
            pltpu.VMEM((D, D), BF), pltpu.VMEM((D, 128), F32),
            pltpu.VMEM((S, D), BF),
            pltpu.SemaphoreType.DMA((3,)),
            pltpu.SemaphoreType.DMA((9,)),
            pltpu.SemaphoreType.DMA((NT,)),
        ],
        compiler_params=pltpu.CompilerParams(vmem_limit_bytes=100 * 1024 * 1024,
                                             disable_semaphore_checks=True),
        name="gmix",
    )(A_x, A_wqkv, A_wo, B_w1, B_w2, B_w3.T, B_w4, gate_w)
```

```python
import jax
import jax.numpy as jnp
from jax import lax
from jax.experimental import pallas as pl
from jax.experimental.pallas import tpu as pltpu

S = 2048
D = 640
F = 1728
TM = 256
T2 = 2 * TM
R1 = 416
NT = S // TM
NL = D // 128
PAD = 8
FM = 1664
BF = jnp.bfloat16
F32 = jnp.float32
EPS = 1e-5

BAND = ((0, 144), (112, 272), (240, 400), (368, 528), (496, 640))


def _dot(a, b):
    return jnp.dot(a, b, preferred_element_type=F32)


def _dot_nt(a, b):
    return lax.dot_general(a, b, (((1,), (1,)), ((), ())), preferred_element_type=F32)


def _gelu(x):
    c = 0.7978845608028654
    t = jnp.tanh(x * (c + (c * 0.044715) * (x * x)))
    return x * (0.5 + 0.5 * t)


def _phi(t):
    return (jnp.maximum(t, 0.0) + 1e-6) + jnp.exp(jnp.minimum(t, 0.0))


def _stats(x):
    m = jnp.mean(x, axis=-1, keepdims=True)
    xc = x - m
    v = jnp.mean(xc * xc, axis=-1, keepdims=True)
    return m, lax.rsqrt(v + EPS)


def _head(idx):
    return (idx * 3277) >> 16


class _Tile:
    pass


def _kernel(ax_hbm, wqkv_hbm, wo_hbm, w1_hbm, w2_hbm, w3t_hbm, w4_hbm, gw_hbm,
            out_hbm,
            xa, wq, wk, wv, wo, w1, w2, w3t, w4, gw_ref, wkT, wqT, gbuf, hbuf, pacc, zacc, mmat, zb, obuf,
            sem_x, sem_w, sem_o):
    def x_cp(n, lo, hi):
        return pltpu.make_async_copy(ax_hbm.at[0, pl.ds(lo, hi - lo), :], xa.at[pl.ds(lo, hi - lo), :], sem_x.at[n])

    x01_cp = x_cp(0, 0, 2 * TM)
    x23_cp = x_cp(1, 2 * TM, 4 * TM)
    x47_cp = x_cp(2, 4 * TM, 8 * TM)
    wq_cp = pltpu.make_async_copy(wqkv_hbm.at[:, pl.ds(0, D)], wq, sem_w.at[0])
    wk_cp = pltpu.make_async_copy(wqkv_hbm.at[:, pl.ds(D, D)], wk, sem_w.at[1])
    wv_cp = pltpu.make_async_copy(wqkv_hbm.at[:, pl.ds(2 * D, D)], wv, sem_w.at[2])
    wo_cp = pltpu.make_async_copy(wo_hbm, wo, sem_w.at[3])
    w1_cp = pltpu.make_async_copy(w1_hbm, w1, sem_w.at[4])
    w2_cp = pltpu.make_async_copy(w2_hbm, w2, sem_w.at[5])
    w3_cp = pltpu.make_async_copy(w3t_hbm, w3t, sem_w.at[6])
    w4_cp = pltpu.make_async_copy(w4_hbm, w4, sem_w.at[7])
    gw_cp = pltpu.make_async_copy(gw_hbm, gw_ref, sem_w.at[8])

    wk_cp.start()
    x01_cp.start()
    gw_cp.start()

    for j in range(NL):
        hbuf[j, 0:PAD, :] = jnp.zeros((PAD, 128), F32)
        hbuf[j, PAD + S:PAD + S + PAD, :] = jnp.zeros((PAD, 128), F32)

    def stage_b(i):
        x = xa[i * TM:(i + 1) * TM, :].astype(F32)
        m, rs = _stats(x)
        s = jnp.sum(x * gw_ref[...].astype(F32).reshape(1, D), axis=-1, keepdims=True)
        g = 0.5 + 0.5 * jnp.tanh(0.5 * s)
        gbuf[i * TM:(i + 1) * TM, :] = jnp.broadcast_to(g, (TM, 128))
        rs = rs + 0.0 * g
        h = _gelu(_dot((x * rs - m * rs).astype(BF), w1[...]))
        for j in range(NL):
            hbuf[j, PAD + i * TM:PAD + (i + 1) * TM, :] = h[:, 128 * j:128 * (j + 1)]

    def stage_k(i):
        pkT = _phi(_dot_nt(wkT[...], xa[i * T2:(i + 1) * T2, :]))
        zp = pkT[:, 0:128]
        for c in range(1, T2 // 128):
            zp = zp + pkT[:, c * 128:(c + 1) * 128]
        if i == 0:
            zacc[...] = zp
        else:
            zacc[...] += zp
        return pkT.astype(BF)

    def stage_p(i, pk, lo=0, hi=D):
        t = _dot(pk, xa[i * T2:(i + 1) * T2, lo:hi])
        if i == 0:
            pacc[:, lo:hi] = t
        else:
            pacc[:, lo:hi] += t

    wk_cp.wait()
    x23_cp.start()
    w1_cp.start()
    wkT[...] = wk[...].T
    x01_cp.wait()
    gw_cp.wait()
    x47_cp.start()
    wq_cp.start()
    wv_cp.start()
    wo_cp.start()
    pk0 = stage_k(0)
    x23_cp.wait()
    w1_cp.wait()
    w2_cp.start()
    w3_cp.start()
    w4_cp.start()
    pk1 = stage_k(1)
    stage_p(0, pk0, 0, 384)
    stage_b(0)
    stage_p(0, pk0, 384, D)
    stage_b(1)
    stage_b(2)
    stage_b(3)
    x47_cp.wait()
    wq_cp.wait()
    wv_cp.wait()
    wo_cp.wait()
    pk2 = stage_k(2)
    stage_p(1, pk1)
    pk3 = stage_k(3)
    wqT[...] = wq[...].T
    stage_p(2, pk2)
    stage_b(4)
    stage_p(3, pk3)
    stage_b(5)

    kvs = []
    for j, (lo, hi) in enumerate(BAND):
        kv = _dot(pacc[lo:hi, :].astype(BF), wv[:, 128 * j:128 * (j + 1)])
        rd = lax.broadcasted_iota(jnp.int32, (hi - lo, 128), 0) + lo
        ce = lax.broadcasted_iota(jnp.int32, (hi - lo, 128), 1) + 128 * j
        kvs.append(jnp.where(_head(rd) == _head(ce), kv, 0.0).astype(BF))
    stage_b(6)
    ms = [_dot(kvs[j], wo[128 * j:128 * (j + 1), :]) for j in range(NL)]
    for j, (lo, hi) in enumerate(BAND):
        a = lo if j == 0 else BAND[j - 1][1]
        b = hi if j == len(BAND) - 1 else BAND[j + 1][0]
        mmat[a:b, :] = ms[j][a - lo:b - lo, :].astype(BF)
        if j + 1 < len(BAND):
            lo2 = BAND[j + 1][0]
            mmat[b:hi, :] = (ms[j][b - lo:hi - lo, :] + ms[j + 1][b - lo2:hi - lo2, :]).astype(BF)
    stage_b(7)
    zb[...] = jnp.broadcast_to(jnp.sum(zacc[...], axis=1, keepdims=True), (D, 128))

    w2_cp.wait()
    w3_cp.wait()
    w4_cp.wait()

    def out_cp(ii, part):
        lo, n = (0, R1) if part == 0 else (R1, T2 - R1)
        r = ii * T2 + lo
        return pltpu.make_async_copy(obuf.at[pl.ds(r, n), :], out_hbm.at[0, pl.ds(r, n), :], sem_o.at[2 * ii + part])

    def f_hs(t):
        lane = lax.broadcasted_iota(jnp.int32, (TM, 128), 1)

        def ld(j, s):
            return hbuf[j, pl.ds(t.r0 + PAD - s, TM), :]

        t.hs = jnp.concatenate([
            ld(0, 1),
            jnp.where(lane < 32, ld(1, 1), ld(1, -1)),
            jnp.where(lane < 64, ld(2, -1), ld(2, 2)),
            jnp.where(lane < 96, ld(3, 2), ld(3, -2)),
            ld(4, -2)], axis=1).astype(BF)

    def f_q(t):
        xat = xa[pl.ds(t.r0, TM), :]
        pq = _phi(_dot_nt(wqT[...], xat))
        tt = pq * jnp.concatenate([zb[...]] * (TM // 128), axis=1)
        sub = lax.broadcasted_iota(jnp.int32, (8, TM), 0)
        parts = []
        for p in range(16):
            v = [tt[40 * p + 8 * i:40 * p + 8 * i + 8, :] for i in range(5)]
            parts.append(v[0] + v[1] + jnp.where(sub < 4, v[2], 0.0))
            parts.append(v[3] + v[4] + jnp.where(sub >= 4, v[2], 0.0))

        def comb(a, b, s):
            lo = (sub & s) == 0
            x = jnp.where(lo, a, b)
            y = jnp.where(lo, b, a)
            if s == 4:
                y = pltpu.roll(y, 4, 0)
            else:
                y = jnp.where(lo, pltpu.roll(y, 8 - s, 0), pltpu.roll(y, s, 0))
            return x + y

        recs = []
        for gi in range(4):
            h = parts[8 * gi:8 * gi + 8]
            l1 = [comb(h[i], h[i + 4], 4) for i in range(4)]
            l2 = [comb(l1[i], l1[i + 2], 2) for i in range(2)]
            recs.append(1.0 / (comb(l2[0], l2[1], 1) + 1e-6))

        def bc(h):
            return jnp.broadcast_to(recs[h // 8][h % 8:h % 8 + 1, :], (8, TM))

        outs = []
        for p in range(16):
            ra, rb = bc(2 * p), bc(2 * p + 1)
            rm = jnp.where(sub < 4, ra, rb)
            v = [pq[40 * p + 8 * i:40 * p + 8 * i + 8, :] for i in range(5)]
            outs += [v[0] * ra, v[1] * ra, v[2] * rm, v[3] * rb, v[4] * rb]
        t.r = jnp.concatenate(outs, axis=0).astype(BF).T

    def f_w2(t):
        t.x1 = xa[pl.ds(t.r0, TM), :].astype(F32) + _dot(t.hs, w2[...])
        m, rs = _stats(t.x1)
        t.ln = (t.x1 * rs - m * rs).astype(BF)

    def f_a(t):
        a = _dot(t.r, mmat[...])
        g = jnp.concatenate([gbuf[pl.ds(t.r0, TM), :]] * NL, axis=1)
        t.omg = 1.0 - g
        t.base = g * a + t.omg * t.x1

    def f_w3(t):
        h2l = _gelu(_dot_nt(w3t[FM:F, :], t.ln)).astype(BF).T
        h2m = _gelu(_dot_nt(t.ln, w3t[0:FM, :])).astype(BF)
        t.h2 = jnp.concatenate([h2m, h2l], axis=1)

    def f_w4(t, r=0, n=TM):
        y = _dot(t.h2[r:r + n, :], w4[...])
        obuf[pl.ds(t.r0 + r, n), :] = (t.base[r:r + n, :] + t.omg[r:r + n, :] * y).astype(BF)

    def body(ii, carry):
        ta, tb = _Tile(), _Tile()
        ta.r0 = pl.multiple_of(ii * T2, T2)
        tb.r0 = pl.multiple_of(ii * T2 + TM, TM)
        f_hs(tb)
        f_w2(tb)
        f_q(tb)
        f_hs(ta)
        f_q(ta)
        f_w2(ta)
        f_a(ta)
        f_w3(ta)
        f_w4(ta)
        f_w3(tb)
        f_a(tb)
        f_w4(tb, 0, R1 - TM)
        out_cp(ii, 0).start()
        f_w4(tb, R1 - TM, T2 - R1)
        out_cp(ii, 1).start()
        return carry

    lax.fori_loop(0, NT // 2, body, 0)
    for j in range(NT // 2):
        out_cp(j, 0).wait()
        out_cp(j, 1).wait()


@jax.jit
def pallas_gated_mix__linear_attn_block__mixer_s_mlp__prompt_kernel(A_x, A_wqkv, A_wo, B_x, B_w1, B_w2, B_w3, B_w4, gate_w):
    del B_x
    hbm = pl.BlockSpec(memory_space=pltpu.HBM)
    return pl.pallas_call(
        _kernel,
        out_shape=jax.ShapeDtypeStruct((1, S, D), BF),
        in_specs=[hbm] * 8,
        out_specs=hbm,
        scratch_shapes=[
            pltpu.VMEM((S, D), BF),
            pltpu.VMEM((D, D), BF), pltpu.VMEM((D, D), BF), pltpu.VMEM((D, D), BF),
            pltpu.VMEM((D, D), BF), pltpu.VMEM((D, D), BF), pltpu.VMEM((D, D), BF),
            pltpu.VMEM((F, D), BF), pltpu.VMEM((F, D), BF),
            pltpu.VMEM((D,), BF),
            pltpu.VMEM((D, D), BF), pltpu.VMEM((D, D), BF),
            pltpu.VMEM((S, 128), F32),
            pltpu.VMEM((NL, S + 2 * PAD, 128), F32),
            pltpu.VMEM((D, D), F32), pltpu.VMEM((D, 128), F32),
            pltpu.VMEM((D, D), BF), pltpu.VMEM((D, 128), F32),
            pltpu.VMEM((S, D), BF),
            pltpu.SemaphoreType.DMA((3,)),
            pltpu.SemaphoreType.DMA((9,)),
            pltpu.SemaphoreType.DMA((NT,)),
        ],
        compiler_params=pltpu.CompilerParams(vmem_limit_bytes=100 * 1024 * 1024,
                                             disable_semaphore_checks=True),
        name="gmix",
    )(A_x, A_wqkv, A_wo, B_w1, B_w2, B_w3.T, B_w4, gate_w)
```
